```python
import os as _os
_os.environ.setdefault("JAX_PLATFORMS", "cpu")
import jax
import jax.numpy as jnp

def _softmax(x, axis=-1):
    return jax.nn.softmax(x, axis=axis)
def _gelu(x):
    return jax.nn.gelu(x, approximate=True)
def _silu(x):
    return jax.nn.silu(x)
def _sigmoid(x):
    return jax.nn.sigmoid(x)
def _layernorm(x, axis=-1, eps=1e-5):
    m = jnp.mean(x, axis=axis, keepdims=True)
    v = jnp.var(x, axis=axis, keepdims=True)
    return (x - m) / jnp.sqrt(v + eps)
def _scatter_add(tgt, idx, src, axis=0):
    return tgt.at[idx].add(src)
def _segment_sum(src, seg, n):
    return jax.ops.segment_sum(src, seg, n)
class _Rng:
    def __init__(self, key):
        self._k = key
    def _next(self):
        self._k, sub = jax.random.split(self._k)
        return sub
    def normal(self, shape):
        return jax.random.normal(self._next(), shape, dtype=jnp.bfloat16)
    def randint(self, lo, hi, shape):
        return jax.random.randint(self._next(), shape, lo, hi, dtype=jnp.int32)
    def uniform(self, shape, lo=0.0, hi=1.0):
        return jax.random.uniform(self._next(), shape, jnp.bfloat16, lo, hi)
    def permutation(self, n):
        return jax.random.permutation(self._next(), n)


kernel_name = 'standalone__gqa_block_cached__near_ridge'

def setup_inputs():
    _rng = _Rng(jax.random.key(int.from_bytes(__import__("os").urandom(4), "little")))
    _w = (lambda a: (lambda t: t.astype(jnp.bfloat16) if jnp.issubdtype(t.dtype, jnp.floating) else t)(jnp.asarray(a)))
    B, Sq, D = 8, 96, 640
    Hq, Hkv, Sk, Dh = 32, 32, 512, 128
    assert Hq % Hkv == 0, (Hq, Hkv)
    return {
        "x": _w((lambda *s: _rng.normal(s) * 0.2)(B, Sq, D)),
        "k_cache": _w((lambda *s: _rng.normal(s) * 3.2)(B, Hkv, Sk, Dh)),
        "v_cache": _w((lambda *s: _rng.normal(s) * 0.05)(B, Hkv, Sk, Dh)),
        "wq": _w((lambda *s: _rng.normal(s) * 0.2)(D, Hq * Dh) * (D ** -0.5)),
        "wo": _w((lambda *s: _rng.normal(s) * 0.05)(Hq * Dh, D) * ((Hq * Dh) ** -0.5)),
    }

def reference(x, k_cache, v_cache, wq, wo):
    B, Sq, D = x.shape
    Hq, Dh = 32, 128
    Hkv = k_cache.shape[1]
    rep = Hq // Hkv
    q = (lambda x, *d: x.transpose(*d))((x @ wq).reshape(B, Sq, Hq, Dh), 0, 2, 1, 3)
    k = jnp.repeat(k_cache, rep, axis=1)
    v = jnp.repeat(v_cache, rep, axis=1)
    scores = jnp.einsum("bhqd,bhkd->bhqk", q, k) * (Dh ** -0.5)
    p = _softmax(scores, axis=-1)
    o = jnp.einsum("bhqk,bhkd->bhqd", p, v)
    return (lambda x, *d: x.transpose(*d))(o, 0, 2, 1, 3).reshape(B, Sq, Hq * Dh) @ wo
```

```python
import jax
import jax.numpy as jnp
from jax import lax
import jax.experimental.pallas as pl
import jax.experimental.pallas.tpu as pltpu


@jax.jit
def pallas_standalone__gqa_block_cached__near_ridge_kernel(
    x: jax.Array,
    k_cache: jax.Array,
    v_cache: jax.Array,
    wq: jax.Array,
    wo: jax.Array,
):
    B, Sq, D = x.shape
    _, Hkv, Sk, Dh = k_cache.shape
    Hq = wq.shape[1] // Dh
    rep = Hq // Hkv
    M = B * Sq
    scale = float(Dh) ** -0.5

    x2 = x.reshape(M, D)

    def kernel(x_ref, k_ref, v_ref, wq_ref, wo_ref, o_ref, q_scr, o_scr, acc_ref):
        h = pl.program_id(0)

        q = jnp.dot(x_ref[...], wq_ref[...], preferred_element_type=jnp.float32)
        q_scr[...] = (q * scale).astype(q_scr.dtype)

        for b in range(B):
            qb = q_scr[b * Sq:(b + 1) * Sq, :]
            s = lax.dot_general(qb, k_ref[b, 0], (((1,), (1,)), ((), ())),
                                preferred_element_type=jnp.float32)
            m = jnp.max(s, axis=-1, keepdims=True)
            p = jnp.exp(s - m)
            l = jnp.sum(p, axis=-1, keepdims=True)
            o = jnp.dot(p.astype(jnp.bfloat16), v_ref[b, 0],
                        preferred_element_type=jnp.float32)
            o_scr[b * Sq:(b + 1) * Sq, :] = (o / l).astype(o_scr.dtype)

        contrib = jnp.dot(o_scr[...], wo_ref[...], preferred_element_type=jnp.float32)

        @pl.when(h == 0)
        def _():
            acc_ref[...] = contrib

        @pl.when(h > 0)
        def _():
            acc_ref[...] += contrib

        @pl.when(h == pl.num_programs(0) - 1)
        def _():
            o_ref[...] = acc_ref[...].astype(o_ref.dtype)

    out = pl.pallas_call(
        kernel,
        grid=(Hq,),
        in_specs=[
            pl.BlockSpec((M, D), lambda h: (0, 0)),
            pl.BlockSpec((B, 1, Sk, Dh), lambda h: (0, h // rep, 0, 0)),
            pl.BlockSpec((B, 1, Sk, Dh), lambda h: (0, h // rep, 0, 0)),
            pl.BlockSpec((D, Dh), lambda h: (0, h)),
            pl.BlockSpec((Dh, D), lambda h: (h, 0)),
        ],
        out_specs=pl.BlockSpec((M, D), lambda h: (0, 0)),
        out_shape=jax.ShapeDtypeStruct((M, D), x.dtype),
        scratch_shapes=[
            pltpu.VMEM((M, Dh), jnp.bfloat16),
            pltpu.VMEM((M, Dh), jnp.bfloat16),
            pltpu.VMEM((M, D), jnp.float32),
        ],
        compiler_params=pltpu.CompilerParams(
            dimension_semantics=("arbitrary",),
            vmem_limit_bytes=64 * 1024 * 1024,
        ),
    )(x2, k_cache, v_cache, wq, wo)
    return out.reshape(B, Sq, D)
```

```python
import jax
import jax.numpy as jnp
from jax import lax
import jax.experimental.pallas as pl
import jax.experimental.pallas.tpu as pltpu

CPH = 2
P = 4
NS = P + 3
NW = 4
TSPLIT = 2
U = 4


@jax.jit
def pallas_standalone__gqa_block_cached__near_ridge_kernel(x, k_cache, v_cache, wq, wo):
    B, Sq, D = x.shape
    _, Hkv, Sk, Dh = k_cache.shape
    Hq = wq.shape[1] // Dh
    rep = Hq // Hkv
    M = B * Sq
    scale = float(Dh) ** -0.5
    CB = B // CPH
    CM = CB * Sq
    T = Hq * CPH
    TB = CB // TSPLIT
    assert T % U == 0 and U % CPH == 0

    x2 = x.reshape(M, D)

    def kernel(x_hbm, k_hbm, v_hbm, wq_hbm, wo_hbm, o_hbm,
               x_v, kbuf, vbuf, wqbuf, wobuf, q_scr, o_scr, p_scr, l_scr, acc_ref, out_v,
               sem_kv, sem_w, sem_x, sem_vt, sem_o, sem_bar):

        def barrier():
            pl.semaphore_signal(sem_bar, 1)
            pl.semaphore_wait(sem_bar, 1)


        def is_static(v):
            return isinstance(v, int)

        def when(cond, fn):
            if isinstance(cond, bool):
                if cond:
                    fn()
            else:
                pl.when(cond)(fn)

        def k_copy(c, j):
            return pltpu.make_async_copy(k_hbm.at[pl.ds(j * CB, CB), (c // CPH) // rep],
                                         kbuf.at[c % NS], sem_kv.at[0, c % NS])

        def v_copy(c, j):
            return pltpu.make_async_copy(v_hbm.at[pl.ds(j * CB, CB), (c // CPH) // rep],
                                         vbuf.at[c % NS], sem_kv.at[1, c % NS])

        def v_tail_copy(g):
            c = T - 1
            j = c % CPH
            return pltpu.make_async_copy(
                v_hbm.at[pl.ds(j * CB + g * TB, TB), (c // CPH) // rep],
                vbuf.at[c % NS, pl.ds(g * TB, TB)], sem_vt.at[g])

        def wq_copy(h):
            off = h * Dh if is_static(h) else pl.multiple_of(h * Dh, Dh)
            return pltpu.make_async_copy(wq_hbm.at[:, pl.ds(off, Dh)],
                                         wqbuf.at[h % NW], sem_w.at[0, h % NW])

        def wo_copy(h):
            off = h * Dh if is_static(h) else pl.multiple_of(h * Dh, Dh)
            return pltpu.make_async_copy(wo_hbm.at[pl.ds(off, Dh), :],
                                         wobuf.at[h % NW], sem_w.at[1, h % NW])

        def out_copy(r0, n, i):
            r = pl.ds(r0, n)
            return pltpu.make_async_copy(out_v.at[r], o_hbm.at[r], sem_o.at[i])

        def issue_need(t, tm):
            j = tm % CPH
            if j == 0:
                when(t + 4 < T, lambda: wq_copy((t + 4) // CPH).start())
            if (tm - 1) % CPH == 0:
                when(t - 1 >= 0, lambda: wo_copy((t - 1) // CPH).start()) if is_static(t) else \
                    wo_copy((t - 1) // CPH).start()
            when(t + 2 < T, lambda: k_copy(t + 2, (tm + 2) % CPH).start())
            if is_static(t) and t == T - 1:
                for g in range(TSPLIT):
                    v_tail_copy(g).start()
            else:
                v_copy(t, j).start()

        def wait_need(t, tm):
            j = tm % CPH
            if j == 0:
                when(t + 4 < T, lambda: wq_copy((t + 4) // CPH).wait())
            if (tm - 1) % CPH == 0:
                when(t - 1 >= 0, lambda: wo_copy((t - 1) // CPH).wait()) if is_static(t) else \
                    wo_copy((t - 1) // CPH).wait()
            when(t + 2 < T, lambda: k_copy(t + 2, (tm + 2) % CPH).wait())
            if not (is_static(t) and t == T - 1):
                v_copy(t, j).wait()

        def q_unit(c, cm, bl):
            rows = pl.ds(((cm % CPH) * CB + bl) * Sq, Sq)
            qn = jnp.dot(x_v[rows, :], wqbuf[(c // CPH) % NW], preferred_element_type=jnp.float32)
            q_scr[cm % U, pl.ds(bl * Sq, Sq), :] = (qn * scale).astype(q_scr.dtype)

        def qk(c, cm, bl):
            return lax.dot_general(q_scr[cm % U, pl.ds(bl * Sq, Sq), :], kbuf[c % NS, bl],
                                   (((1,), (1,)), ((), ())), preferred_element_type=jnp.float32)

        def softmax_store(s, cm, bl):
            r = pl.ds(bl * Sq, Sq)
            m = jnp.max(s, axis=-1, keepdims=True)
            p = jnp.exp(s - m)
            l_scr[cm % U, r, :] = jnp.sum(p, axis=-1, keepdims=True)
            p_scr[cm % U, r, :] = p.astype(p_scr.dtype)

        def pv(c, cm, bl):
            r = pl.ds(bl * Sq, Sq)
            o = jnp.dot(p_scr[cm % U, r, :], vbuf[c % NS, bl], preferred_element_type=jnp.float32)
            return (o / l_scr[cm % U, r, :]).astype(jnp.bfloat16)

        def o_unit(c, cm, bl, ob, final):
            rows = pl.ds(((cm % CPH) * CB + bl) * Sq, Sq)
            contrib = jnp.dot(ob, wobuf[(c // CPH) % NW], preferred_element_type=jnp.float32)
            if final:
                out_v[rows, :] = (acc_ref[rows, :] + contrib).astype(out_v.dtype)
            else:
                acc_ref[rows, :] += contrib

        x_copy = pltpu.make_async_copy(x_hbm, x_v, sem_x.at[0])
        x_copy.start()
        barrier()
        wq_copy(0).start()
        barrier()
        wq_copy(1).start()
        barrier()
        k_copy(0, 0).start()
        barrier()
        k_copy(1, 1 % CPH).start()
        for t in range(P):
            barrier()
            issue_need(t, t % U)
        barrier()

        acc_ref[...] = jnp.zeros_like(acc_ref)
        x_copy.wait()
        wq_copy(0).wait()
        wq_copy(1).wait()
        for c in range(4):
            for bl in range(CB):
                q_unit(c, c, bl)
        for c in range(2):
            k_copy(c, c % CPH).wait()
            for bl in range(CB):
                softmax_store(qk(c, c, bl), c, bl)

        def chunk_body(t, tm):
            st = is_static(t)
            when(t + P < T, lambda: issue_need(t + P, (tm + P) % U)) if st else None
            if not st:
                issue_need(t + P, (tm + P) % U)
            wait_need(t, tm)
            do_q = (t + 4 < T) if st else True
            do_k = (t + 2 < T) if st else True
            do_o = (t - 1 >= 0) if st else True
            last = st and t == T - 1
            final_o = st and (t - 1) // CPH == Hq - 1
            if last:
                for bl in range(CB):
                    o_unit(t - 1, tm - 1, bl, o_scr[(tm - 1) % U, pl.ds(bl * Sq, Sq), :], final_o)
                out_copy(((tm - 1) % CPH) * CM, CM, 0).start()
                for g in range(TSPLIT):
                    v_tail_copy(g).wait()
                    for bl in range(g * TB, (g + 1) * TB):
                        o_unit(t, tm, bl, pv(t, tm, bl), True)
                    out_copy((tm % CPH) * CM + g * TB * Sq, TB * Sq, 1 + g).start()
                return
            for bl in range(CB):
                if do_k:
                    s = qk(t + 2, tm + 2, bl)
                if do_q:
                    q_unit(t + 4, tm + 4, bl)
                o_new = pv(t, tm, bl)
                if do_k:
                    softmax_store(s, tm + 2, bl)
                if do_o:
                    o_unit(t - 1, tm - 1, bl, o_scr[(tm - 1) % U, pl.ds(bl * Sq, Sq), :], final_o)
                o_scr[tm % U, pl.ds(bl * Sq, Sq), :] = o_new

        NPEEL_END = ((P + 4 + U - 1) // U) * U
        for t in range(U):
            chunk_body(t, t)

        def loop_body(i, carry):
            for u in range(U):
                chunk_body(i * U + u, u)
            return carry

        lax.fori_loop(1, (T - NPEEL_END) // U, loop_body, 0)
        for t in range(T - NPEEL_END, T):
            chunk_body(t, t % U)

        out_copy(((T - 2) % CPH) * CM, CM, 0).wait()
        for g in range(TSPLIT):
            out_copy(((T - 1) % CPH) * CM + g * TB * Sq, TB * Sq, 1 + g).wait()

    out = pl.pallas_call(
        kernel,
        in_specs=[pl.BlockSpec(memory_space=pl.ANY)] * 5,
        out_specs=pl.BlockSpec(memory_space=pl.ANY),
        out_shape=jax.ShapeDtypeStruct((M, D), x.dtype),
        scratch_shapes=[
            pltpu.VMEM((M, D), jnp.bfloat16),
            pltpu.VMEM((NS, CB, Sk, Dh), jnp.bfloat16),
            pltpu.VMEM((NS, CB, Sk, Dh), jnp.bfloat16),
            pltpu.VMEM((NW, D, Dh), jnp.bfloat16),
            pltpu.VMEM((NW, Dh, D), jnp.bfloat16),
            pltpu.VMEM((U, CM, Dh), jnp.bfloat16),
            pltpu.VMEM((U, CM, Dh), jnp.bfloat16),
            pltpu.VMEM((U, CM, Sk), jnp.bfloat16),
            pltpu.VMEM((U, CM, 1), jnp.float32),
            pltpu.VMEM((M, D), jnp.float32),
            pltpu.VMEM((M, D), jnp.bfloat16),
            pltpu.SemaphoreType.DMA((2, NS)),
            pltpu.SemaphoreType.DMA((2, NW)),
            pltpu.SemaphoreType.DMA((1,)),
            pltpu.SemaphoreType.DMA((TSPLIT,)),
            pltpu.SemaphoreType.DMA((1 + TSPLIT,)),
            pltpu.SemaphoreType.REGULAR,
        ],
        compiler_params=pltpu.CompilerParams(
            vmem_limit_bytes=64 * 1024 * 1024,
        ),
    )(x2, k_cache, v_cache, wq, wo)
    return out.reshape(B, Sq, D)
```

```python
import jax
import jax.numpy as jnp
from jax import lax
import jax.experimental.pallas as pl
import jax.experimental.pallas.tpu as pltpu

CPH = 2
P = 4
NS = P + 3
NW = 4
TSPLIT = 2
U = 4


@jax.jit
def pallas_standalone__gqa_block_cached__near_ridge_kernel(x, k_cache, v_cache, wq, wo):
    B, Sq, D = x.shape
    _, Hkv, Sk, Dh = k_cache.shape
    Hq = wq.shape[1] // Dh
    rep = Hq // Hkv
    M = B * Sq
    scale = float(Dh) ** -0.5
    CB = B // CPH
    CM = CB * Sq
    T = Hq * CPH
    TB = CB // TSPLIT
    assert B % CPH == 0 and CB % TSPLIT == 0
    assert T % U == 0 and U % CPH == 0

    x2 = x.reshape(M, D)

    def kernel(x_hbm, k_hbm, v_hbm, wq_hbm, wo_hbm, o_hbm,
               x_v, kbuf, vbuf, wqbuf, wobuf, q_scr, o_scr, p_scr, l_scr, acc_ref, out_v,
               sem_kv, sem_w, sem_x, sem_vt, sem_o, sem_bar):

        def barrier():
            pl.semaphore_signal(sem_bar, 1)
            pl.semaphore_wait(sem_bar, 1)

        def is_static(v):
            return isinstance(v, int)

        def when(cond, fn):
            if isinstance(cond, bool):
                if cond:
                    fn()
            else:
                pl.when(cond)(fn)

        def k_copy(c, j):
            return pltpu.make_async_copy(k_hbm.at[pl.ds(j * CB, CB), (c // CPH) // rep],
                                         kbuf.at[c % NS], sem_kv.at[0, c % NS])

        def v_copy(c, j):
            return pltpu.make_async_copy(v_hbm.at[pl.ds(j * CB, CB), (c // CPH) // rep],
                                         vbuf.at[c % NS], sem_kv.at[1, c % NS])

        def v_tail_copy(g):
            c = T - 1
            j = c % CPH
            return pltpu.make_async_copy(
                v_hbm.at[pl.ds(j * CB + g * TB, TB), (c // CPH) // rep],
                vbuf.at[c % NS, pl.ds(g * TB, TB)], sem_vt.at[g])

        def wq_copy(h):
            off = h * Dh if is_static(h) else pl.multiple_of(h * Dh, Dh)
            return pltpu.make_async_copy(wq_hbm.at[:, pl.ds(off, Dh)],
                                         wqbuf.at[h % NW], sem_w.at[0, h % NW])

        def wo_copy(h):
            off = h * Dh if is_static(h) else pl.multiple_of(h * Dh, Dh)
            return pltpu.make_async_copy(wo_hbm.at[pl.ds(off, Dh), :],
                                         wobuf.at[h % NW], sem_w.at[1, h % NW])

        def out_copy(r0, n, i):
            r = pl.ds(r0, n)
            return pltpu.make_async_copy(out_v.at[r], o_hbm.at[r], sem_o.at[i])

        def issue_need(t, tm):
            j = tm % CPH
            if j == 0:
                when(t + 4 < T, lambda: wq_copy((t + 4) // CPH).start())
                barrier()
            if (tm - 1) % CPH == 0:
                when(t - 1 >= 0, lambda: wo_copy((t - 1) // CPH).start())
                barrier()
            when(t + 2 < T, lambda: k_copy(t + 2, (tm + 2) % CPH).start())
            barrier()
            if is_static(t) and t == T - 1:
                for g in range(TSPLIT):
                    v_tail_copy(g).start()
                    barrier()
            else:
                v_copy(t, j).start()

        def wait_need(t, tm):
            j = tm % CPH
            if j == 0:
                when(t + 4 < T, lambda: wq_copy((t + 4) // CPH).wait())
            if (tm - 1) % CPH == 0:
                when(t - 1 >= 0, lambda: wo_copy((t - 1) // CPH).wait())
            when(t + 2 < T, lambda: k_copy(t + 2, (tm + 2) % CPH).wait())
            if not (is_static(t) and t == T - 1):
                v_copy(t, j).wait()

        def q_unit(c, cm, bl):
            rows = pl.ds(((cm % CPH) * CB + bl) * Sq, Sq)
            qn = jnp.dot(x_v[rows, :], wqbuf[(c // CPH) % NW], preferred_element_type=jnp.float32)
            q_scr[cm % U, pl.ds(bl * Sq, Sq), :] = (qn * scale).astype(q_scr.dtype)

        def qk(c, cm, bl):
            return lax.dot_general(q_scr[cm % U, pl.ds(bl * Sq, Sq), :], kbuf[c % NS, bl],
                                   (((1,), (1,)), ((), ())), preferred_element_type=jnp.float32)

        def softmax_store(s, cm, bl):
            r = pl.ds(bl * Sq, Sq)
            m = jnp.max(s, axis=-1, keepdims=True)
            p = jnp.exp(s - m)
            l_scr[cm % U, r, :] = jnp.sum(p, axis=-1, keepdims=True)
            p_scr[cm % U, r, :] = p.astype(p_scr.dtype)

        def pv(c, cm, bl):
            r = pl.ds(bl * Sq, Sq)
            o = jnp.dot(p_scr[cm % U, r, :], vbuf[c % NS, bl], preferred_element_type=jnp.float32)
            return (o / l_scr[cm % U, r, :]).astype(jnp.bfloat16)

        def o_unit(c, cm, bl, ob, final):
            rows = pl.ds(((cm % CPH) * CB + bl) * Sq, Sq)
            contrib = jnp.dot(ob, wobuf[(c // CPH) % NW], preferred_element_type=jnp.float32)
            if final:
                out_v[rows, :] = (acc_ref[rows, :] + contrib).astype(out_v.dtype)
            else:
                acc_ref[rows, :] += contrib

        x_copy = pltpu.make_async_copy(x_hbm, x_v, sem_x.at[0])
        x_copy.start()
        barrier()
        wq_copy(0).start()
        barrier()
        wq_copy(1).start()
        barrier()
        k_copy(0, 0).start()
        barrier()
        k_copy(1, 1 % CPH).start()
        for t in range(P):
            barrier()
            issue_need(t, t % U)
        barrier()

        acc_ref[...] = jnp.zeros_like(acc_ref)
        x_copy.wait()
        wq_copy(0).wait()
        wq_copy(1).wait()
        for c in range(4):
            for bl in range(CB):
                q_unit(c, c, bl)
        for c in range(2):
            k_copy(c, c % CPH).wait()
            for bl in range(CB):
                softmax_store(qk(c, c, bl), c, bl)

        def chunk_body(t, tm):
            st = is_static(t)
            if st:
                if t + P < T:
                    issue_need(t + P, (tm + P) % U)
            else:
                issue_need(t + P, (tm + P) % U)
            wait_need(t, tm)
            do_q = (t + 4 < T) if st else True
            do_k = (t + 2 < T) if st else True
            do_o = (t - 1 >= 0) if st else True
            final_o = st and (t - 1) // CPH == Hq - 1
            if st and t == T - 1:
                for bl in range(CB):
                    o_unit(t - 1, tm - 1, bl, o_scr[(tm - 1) % U, pl.ds(bl * Sq, Sq), :], final_o)
                out_copy(((tm - 1) % CPH) * CM, CM, 0).start()
                for g in range(TSPLIT):
                    v_tail_copy(g).wait()
                    for bl in range(g * TB, (g + 1) * TB):
                        o_unit(t, tm, bl, pv(t, tm, bl), True)
                    out_copy((tm % CPH) * CM + g * TB * Sq, TB * Sq, 1 + g).start()
                return
            for bl in range(CB):
                if do_k:
                    s = qk(t + 2, tm + 2, bl)
                if do_q:
                    q_unit(t + 4, tm + 4, bl)
                o_new = pv(t, tm, bl)
                if do_k:
                    softmax_store(s, tm + 2, bl)
                if do_o:
                    o_unit(t - 1, tm - 1, bl, o_scr[(tm - 1) % U, pl.ds(bl * Sq, Sq), :], final_o)
                o_scr[tm % U, pl.ds(bl * Sq, Sq), :] = o_new

        n_end = ((P + 4 + U - 1) // U) * U
        for t in range(U):
            chunk_body(t, t)

        def loop_body(i, carry):
            for u in range(U):
                chunk_body(i * U + u, u)
            return carry

        lax.fori_loop(1, (T - n_end) // U, loop_body, 0)
        for t in range(T - n_end, T):
            chunk_body(t, t % U)

        out_copy(((T - 2) % CPH) * CM, CM, 0).wait()
        for g in range(TSPLIT):
            out_copy(((T - 1) % CPH) * CM + g * TB * Sq, TB * Sq, 1 + g).wait()

    out = pl.pallas_call(
        kernel,
        in_specs=[pl.BlockSpec(memory_space=pl.ANY)] * 5,
        out_specs=pl.BlockSpec(memory_space=pl.ANY),
        out_shape=jax.ShapeDtypeStruct((M, D), x.dtype),
        scratch_shapes=[
            pltpu.VMEM((M, D), jnp.bfloat16),
            pltpu.VMEM((NS, CB, Sk, Dh), jnp.bfloat16),
            pltpu.VMEM((NS, CB, Sk, Dh), jnp.bfloat16),
            pltpu.VMEM((NW, D, Dh), jnp.bfloat16),
            pltpu.VMEM((NW, Dh, D), jnp.bfloat16),
            pltpu.VMEM((U, CM, Dh), jnp.bfloat16),
            pltpu.VMEM((U, CM, Dh), jnp.bfloat16),
            pltpu.VMEM((U, CM, Sk), jnp.bfloat16),
            pltpu.VMEM((U, CM, 1), jnp.float32),
            pltpu.VMEM((M, D), jnp.float32),
            pltpu.VMEM((M, D), jnp.bfloat16),
            pltpu.SemaphoreType.DMA((2, NS)),
            pltpu.SemaphoreType.DMA((2, NW)),
            pltpu.SemaphoreType.DMA((1,)),
            pltpu.SemaphoreType.DMA((TSPLIT,)),
            pltpu.SemaphoreType.DMA((1 + TSPLIT,)),
            pltpu.SemaphoreType.REGULAR,
        ],
        compiler_params=pltpu.CompilerParams(
            vmem_limit_bytes=64 * 1024 * 1024,
        ),
    )(x2, k_cache, v_cache, wq, wo)
    return out.reshape(B, Sq, D)
```
